```python
import os as _os
_os.environ.setdefault("JAX_PLATFORMS", "cpu")
import jax
import jax.numpy as jnp

def _softmax(x, axis=-1):
    return jax.nn.softmax(x, axis=axis)
def _gelu(x):
    return jax.nn.gelu(x, approximate=True)
def _silu(x):
    return jax.nn.silu(x)
def _sigmoid(x):
    return jax.nn.sigmoid(x)
def _layernorm(x, axis=-1, eps=1e-5):
    m = jnp.mean(x, axis=axis, keepdims=True)
    v = jnp.var(x, axis=axis, keepdims=True)
    return (x - m) / jnp.sqrt(v + eps)
def _scatter_add(tgt, idx, src, axis=0):
    return tgt.at[idx].add(src)
def _segment_sum(src, seg, n):
    return jax.ops.segment_sum(src, seg, n)
class _Rng:
    def __init__(self, key):
        self._k = key
    def _next(self):
        self._k, sub = jax.random.split(self._k)
        return sub
    def normal(self, shape):
        return jax.random.normal(self._next(), shape, dtype=jnp.bfloat16)
    def randint(self, lo, hi, shape):
        return jax.random.randint(self._next(), shape, lo, hi, dtype=jnp.int32)
    def uniform(self, shape, lo=0.0, hi=1.0):
        return jax.random.uniform(self._next(), shape, jnp.bfloat16, lo, hi)
    def permutation(self, n):
        return jax.random.permutation(self._next(), n)


kernel_name = 'standalone__mha_block_cached__near_ridge'

def setup_inputs():
    _rng = _Rng(jax.random.key(int.from_bytes(__import__("os").urandom(4), "little")))
    _w = (lambda a: (lambda t: t.astype(jnp.bfloat16) if jnp.issubdtype(t.dtype, jnp.floating) else t)(jnp.asarray(a)))
    B, Sq, D = 8, 96, 576
    H, Sk, Dh = 32, 96, 128
    return {
        "x": _w((lambda *s: _rng.normal(s) * 0.8)(B, Sq, D)),
        "k_cache": _w((lambda *s: _rng.normal(s) * 0.8)(B, H, Sk, Dh)),
        "v_cache": _w((lambda *s: _rng.normal(s) * 0.05)(B, H, Sk, Dh)),
        "wq": _w((lambda *s: _rng.normal(s) * 0.8)(D, H * Dh) * (D ** -0.5)),
        "wo": _w((lambda *s: _rng.normal(s) * 0.05)(H * Dh, D) * ((H * Dh) ** -0.5)),
    }

def reference(x, k_cache, v_cache, wq, wo):
    B, Sq, D = x.shape
    H, Dh = 32, 128
    q = (lambda x, *d: x.transpose(*d))((x @ wq).reshape(B, Sq, H, Dh), 0, 2, 1, 3)
    scores = jnp.einsum("bhqd,bhkd->bhqk", q, k_cache) * (Dh ** -0.5)
    p = _softmax(scores, axis=-1)
    o = jnp.einsum("bhqk,bhkd->bhqd", p, v_cache)
    return (lambda x, *d: x.transpose(*d))(o, 0, 2, 1, 3).reshape(B, Sq, H * Dh) @ wo
```

```python
import jax
import jax.numpy as jnp
import jax.experimental.pallas as pl
import jax.experimental.pallas.tpu as pltpu
from jax import lax

G = 4
LOG2E = 1.4426950408889634
NT = (((1,), (1,)), ((), ()))
OROWS = [(0,288),(288,576)]

@jax.jit
def pallas_standalone__mha_block_cached__near_ridge_kernel(x, k_cache, v_cache, wq, wo):
    B, Sq, D = x.shape
    _, H, Sk, Dh = k_cache.shape
    M = B * Sq
    NG = H // G
    GW = G * Dh
    TT = 128
    NTT = M // TT
    c = (Dh ** -0.5) * LOG2E
    f32, bf16 = jnp.float32, jnp.bfloat16
    XCH = [(0, 2), (2, 6), (6, 8)]

    def kernel(x_hbm, k_hbm, v_hbm, wq_hbm, wo_hbm, o_hbm,
               x_v, k_v, v_v, wq_v, wo_v, q_s, a_s, acc, o_v, sx, sq, sk, sv, so, sout):
        def cp_x(i):
            lo, hi = XCH[i]
            return pltpu.make_async_copy(x_hbm.at[lo*Sq:hi*Sq], x_v.at[lo*Sq:hi*Sq], sx.at[i])
        def cp_q(g):
            return pltpu.make_async_copy(wq_hbm.at[:, g*GW:(g+1)*GW], wq_v.at[g], sq.at[g])
        def cp_o(g):
            return pltpu.make_async_copy(wo_hbm.at[:, g*GW:(g+1)*GW], wo_v.at[g], so.at[g])
        def cp_k(g):
            return pltpu.make_async_copy(k_hbm.at[:, g*G:(g+1)*G], k_v.at[g], sk.at[g])
        def cp_v(g):
            return pltpu.make_async_copy(v_hbm.at[:, g*G:(g+1)*G], v_v.at[g], sv.at[g])
        def cp_out(j):
            return pltpu.make_async_copy(o_v.at[pl.ds(j * TT, TT)], o_hbm.at[pl.ds(j * TT, TT)], sout.at[j])

        def qproj(g, b):
            q_s[g, b*Sq:(b+1)*Sq, :] = jnp.dot(x_v[b*Sq:(b+1)*Sq, :], wq_v[g], preferred_element_type=f32).astype(bf16)

        def scores(g, b):
            res = []
            for h in range(G):
                q = q_s[g, b*Sq:(b+1)*Sq, h*Dh:(h+1)*Dh]
                s = lax.dot_general(q, k_v[g, b, h], NT, preferred_element_type=f32)
                m = jnp.max(s, axis=-1, keepdims=True)
                e = jnp.exp2((s - m) * c)
                l = jnp.sum(e, axis=-1, keepdims=True)
                r = pl.reciprocal(l, approx=True)
                r = r * (2.0 - l * r)
                res.append((e.astype(bf16), r))
            return res
        def pv(g, b, res):
            for h in range(G):
                e, r = res[h]
                o = jnp.dot(e, v_v[g, b, h], preferred_element_type=f32)
                a_s[g, b*Sq:(b+1)*Sq, h*Dh:(h+1)*Dh] = (o * r).astype(bf16)

        pieces = [(j, lo, hi) for j in range(NTT) for lo, hi in OROWS]
        def oproj(g, piece):
            j, lo, hi = pieces[piece]
            r = lax.dot_general(wo_v[g, lo:hi, :], a_s[g, j*TT:(j+1)*TT, :], NT, preferred_element_type=f32)
            if g == 0:
                acc[lo:hi, j*TT:(j+1)*TT] = r
            else:
                acc[lo:hi, j*TT:(j+1)*TT] += r
            if g == NG-1 and hi == D:
                o_v[j*TT:(j+1)*TT, :] = acc[:, j*TT:(j+1)*TT].T.astype(bf16)
                cp_out(j).start()
        NP = len(pieces)
        def stage(ga, go):
            for b in range(B):
                if ga is not None: res = scores(ga, b)
                if go is not None:
                    for piece in range(b*NP//B, (b+1)*NP//B):
                        oproj(go, piece)
                if ga is not None: pv(ga, b, res)

        cp_x(0).start(); cp_q(0).start()
        cp_x(1).start(); cp_x(2).start(); cp_q(1).start()
        cp_x(0).wait(); cp_q(0).wait()
        cp_q(2).start()
        qproj(0, 0); qproj(0, 1)
        cp_x(1).wait()
        cp_q(3).start(); cp_q(4).start()
        for b in range(2, 6): qproj(0, b)
        cp_x(2).wait(); cp_q(1).wait()
        for g in range(5, NG): cp_q(g).start()
        cp_k(0).start(); cp_v(0).start(); cp_o(0).start(); cp_k(1).start(); cp_v(1).start(); cp_o(1).start()
        for b in range(6, 8): qproj(0, b)
        for b in range(B): qproj(1, b)
        cp_q(2).wait(); cp_q(3).wait()
        for g in range(2, 5):
            cp_k(g).start(); cp_v(g).start(); cp_o(g).start()
        for g in (2, 3):
            for b in range(B): qproj(g, b)
        for g in range(4, NG): cp_q(g).wait()
        for g in range(5, NG):
            cp_k(g).start(); cp_v(g).start(); cp_o(g).start()
        for g in range(4, NG-1):
            for b in range(B): qproj(g, b)
        for g in range(0, 4):
            cp_k(g).wait(); cp_v(g).wait(); cp_o(g).wait()
        for b in range(B):
            res = scores(0, b)
            qproj(NG-1, b)
            pv(0, b, res)
        for g in range(1, 4):
            stage(g, g-1)
        for g in range(4, NG):
            cp_k(g).wait(); cp_v(g).wait(); cp_o(g).wait()
        for g in range(4, NG):
            stage(g, g-1)
        stage(None, NG-1)
        for j in range(NTT):
            cp_out(j).wait()

    any_spec = pl.BlockSpec(memory_space=pltpu.HBM)
    out = pl.pallas_call(
        kernel,
        in_specs=[any_spec] * 5,
        out_specs=any_spec,
        out_shape=jax.ShapeDtypeStruct((M, D), x.dtype),
        scratch_shapes=[
            pltpu.VMEM((M, D), bf16),
            pltpu.VMEM((NG, B, G, Sk, Dh), bf16),
            pltpu.VMEM((NG, B, G, Sk, Dh), bf16),
            pltpu.VMEM((NG, D, GW), bf16),
            pltpu.VMEM((NG, D, GW), bf16),
            pltpu.VMEM((NG, M, GW), bf16),
            pltpu.VMEM((NG, M, GW), bf16),
            pltpu.VMEM((D, M), f32),
            pltpu.VMEM((M, D), bf16),
            pltpu.SemaphoreType.DMA((3,)),
            pltpu.SemaphoreType.DMA((NG,)),
            pltpu.SemaphoreType.DMA((NG,)),
            pltpu.SemaphoreType.DMA((NG,)),
            pltpu.SemaphoreType.DMA((NG,)),
            pltpu.SemaphoreType.DMA((NTT,)),
        ],
        compiler_params=pltpu.CompilerParams(vmem_limit_bytes=100*1024*1024),
    )(x.reshape(M, D), k_cache, v_cache, wq, wo.T)
    return out.reshape(B, Sq, D)
```

```python
import jax
import jax.numpy as jnp
import jax.experimental.pallas as pl
import jax.experimental.pallas.tpu as pltpu
from jax import lax

G = 4
TT = 128
LOG2E = 1.4426950408889634
NT = (((1,), (1,)), ((), ()))

MAIN = ("q00 S00 q01 S01 q02 V00 V01 S02 o000 V02 S03 q03 V03 S04 o001 V04 S05 q04 V05 S06 o010 V06 "
        "S07 o011 V07 o020 q05 o021 o030 q06 o031 o040 q07 o041 o050 o051")
POST = ("S00 S01 S02 S03 S04 S05 S06 V00 S07 V01 S10 o000 V02 V03 o001 V04 S11 o010 V05 S12 o011 V06 "
        "o020 V07 V10 S13 o021 V11 S14 o030 V12 S15 o031 V13 S16 o040 V14 S17 o041 V15 o050 V16 o051 V17 "
        "f100 f101 f110 f111 w10 f120 f121 w11 f130 f131 w12 f140 f141 w13 f150 w14 f151")


@jax.jit
def pallas_standalone__mha_block_cached__near_ridge_kernel(x, k_cache, v_cache, wq, wo):
    B, Sq, D = x.shape
    _, H, Sk, Dh = k_cache.shape
    M = B * Sq
    NG, GW, NTT = H // G, G * Dh, M // TT
    NIT = NG - 2
    assert (B, Sq, D, H * Dh) == (8, 96, 576, 4096)
    o_rows = [(0, 288), (288, 576)]
    f_rows = [[(0, 256)], [(256, 512), (512, 576)]]
    f_cols = [(0, 384), (384, 576)]
    c = (Dh ** -0.5) * LOG2E
    f32, bf16 = jnp.float32, jnp.bfloat16

    def kernel(x_hbm, k_hbm, v_hbm, wq_hbm, wo_hbm, o_hbm,
               x_v, k_v, v_v, wq_v, wo_v, q_s, a_s, acc, sem):
        copy = pltpu.make_async_copy

        def cols(g):
            return pl.ds(g * GW, GW) if isinstance(g, int) else pl.ds(pl.multiple_of(g * GW, GW), GW)

        def cx(lo, hi, s):
            return [copy(x_hbm.at[lo * Sq:hi * Sq], x_v.at[lo * Sq:hi * Sq], sem.at[s])]

        def cq(g, s):
            return [copy(wq_hbm.at[:, cols(g)], wq_v.at[g], sem.at[s])]

        def ckvo(g, s):
            return [copy(k_hbm.at[:, pl.ds(g * G, G)], k_v.at[g], sem.at[s]),
                    copy(v_hbm.at[:, pl.ds(g * G, G)], v_v.at[g], sem.at[s]),
                    copy(wo_hbm.at[:, cols(g)], wo_v.at[g], sem.at[s])]

        def start(cs):
            for cp in cs:
                cp.start()

        def wait(cs):
            for cp in cs:
                cp.wait()

        def qproj(g, b):
            rows = slice(b * Sq, (b + 1) * Sq)
            q_s[g, rows, :] = jnp.dot(x_v[rows, :], wq_v[g], preferred_element_type=f32).astype(bf16)

        def scores(g, b):
            res = []
            for h in range(G):
                q = q_s[g, b * Sq:(b + 1) * Sq, h * Dh:(h + 1) * Dh]
                s = lax.dot_general(q, k_v[g, b, h], NT, preferred_element_type=f32)
                m = jnp.max(s, axis=-1, keepdims=True)
                e = jnp.exp2((s - m) * c)
                l = jnp.sum(e, axis=-1, keepdims=True)
                r = pl.reciprocal(l, approx=True)
                r = r * (2.0 - l * r)
                res.append((e.astype(bf16), r))
            return res

        def pv(g, b, res, slot):
            for h in range(G):
                e, r = res[h]
                o = jnp.dot(e, v_v[g, b, h], preferred_element_type=f32)
                a_s[slot, b * Sq:(b + 1) * Sq, h * Dh:(h + 1) * Dh] = (o * r).astype(bf16)

        def attn_tile(slot, j):
            return a_s[slot, j * TT:(j + 1) * TT, 0:GW]

        def run(prog, g0, zero=None):
            res, pend, outs = {}, {}, []

            def emit(j, lo, hi):
                rows = pl.ds(pl.multiple_of((zero + j) * TT, TT), TT)
                outs.append(copy(a_s.at[2, rows, lo:hi], o_hbm.at[pl.ds(j * TT, TT), lo:hi], sem.at[0]))
                outs[-1].start()

            def stage_out(j, lo, hi, val):
                a_s[2, pl.ds(pl.multiple_of((zero + j) * TT, TT), TT), lo:hi] = val.astype(bf16)

            for t in prog.split():
                op, d, i = t[0], int(t[1]), int(t[2])
                g = g0 + d
                tile = slice(i * TT, (i + 1) * TT)
                if op == 'q':
                    qproj(g + 2, i)
                elif op == 'S':
                    res[t[1:]] = scores(g, i)
                elif op == 'V':
                    pv(g, i, res.pop(t[1:]), d)
                elif op == 'o':
                    lo, hi = o_rows[int(t[3])]
                    acc[lo:hi, tile] += lax.dot_general(
                        wo_v[g, lo:hi, :], attn_tile(d, i), NT, preferred_element_type=f32)
                elif op == 'f' and i < NTT - 1:
                    for lo, hi in f_rows[int(t[3])]:
                        r = lax.dot_general(wo_v[g, lo:hi, :], attn_tile(d, i), NT, preferred_element_type=f32)
                        pend.setdefault(i, []).append((lo, hi, (acc[lo:hi, tile] + r).T))
                elif op == 'f':
                    lo, hi = f_cols[int(t[3])]
                    r = lax.dot_general(attn_tile(d, i), wo_v[g, lo:hi, :], NT, preferred_element_type=f32)
                    stage_out(i, lo, hi, acc[lo:hi, tile].T + r)
                    emit(i, lo, hi)
                elif op == 'w':
                    for lo, hi, val in pend.pop(i):
                        stage_out(i, lo, hi, val)
                    emit(i, 0, D)
            return outs

        def stage(i):
            return cq(i + 2, 5 + i) + ckvo(i, 5 + i)

        d0 = cq(0, 0) + cx(0, 1, 0)
        d1 = cx(1, 3, 1)
        d2 = cx(3, B, 2)
        d3 = cq(1, 3)
        dl = ckvo(NG - 2, 4) + ckvo(NG - 1, 4)
        start(d0 + d1 + d2 + d3)
        for i in range(NIT):
            start(stage(i))
        start(dl)

        @pl.loop(0, D // 48)
        def _(i):
            acc[pl.ds(pl.multiple_of(i * 48, 48), 48), :] = jnp.zeros((48, M), f32)

        for cs, lo, hi in ((d0, 0, 1), (d1, 1, 3), (d2, 3, B)):
            wait(cs)
            for b in range(lo, hi):
                qproj(0, b)
        wait(d3)
        for b in range(B):
            qproj(1, b)

        def body(i):
            wait(stage(i))
            run(MAIN, i)
            return i + 1

        zero = lax.while_loop(lambda i: i < NIT, body, 0) - NIT
        wait(dl)
        wait(run(POST, NG - 2, zero))

    hbm = pl.BlockSpec(memory_space=pltpu.HBM)
    out = pl.pallas_call(
        kernel,
        in_specs=[hbm] * 5,
        out_specs=hbm,
        out_shape=jax.ShapeDtypeStruct((M, D), x.dtype),
        scratch_shapes=[
            pltpu.VMEM((M, D), bf16),
            pltpu.VMEM((NG, B, G, Sk, Dh), bf16),
            pltpu.VMEM((NG, B, G, Sk, Dh), bf16),
            pltpu.VMEM((NG, D, GW), bf16),
            pltpu.VMEM((NG, D, GW), bf16),
            pltpu.VMEM((NG, M, GW), bf16),
            pltpu.VMEM((3, M, D), bf16),
            pltpu.VMEM((D, M), f32),
            pltpu.SemaphoreType.DMA((5 + NIT,)),
        ],
        compiler_params=pltpu.CompilerParams(vmem_limit_bytes=100 * 1024 * 1024),
    )(x.reshape(M, D), k_cache, v_cache, wq, wo.T)
    return out.reshape(B, Sq, D)
```
